```python
import jax
import jax.numpy as jnp

def _softmax(x, axis=-1):
    return jax.nn.softmax(x, axis=axis)

def _gelu(x):
    return jax.nn.gelu(x, approximate=True)

def _silu(x):
    return jax.nn.silu(x)

def _sigmoid(x):
    return jax.nn.sigmoid(x)

def _layernorm(x, axis=-1, eps=1e-05):
    m = jnp.mean(x, axis=axis, keepdims=True)
    v = jnp.var(x, axis=axis, keepdims=True)
    return (x - m) / jnp.sqrt(v + eps)

def _scatter_add(tgt, idx, src, axis=0):
    return tgt.at[idx].add(src)

def _segment_sum(src, seg, n):
    return jax.ops.segment_sum(src, seg, n)

class _Rng:

    def __init__(self, key):
        self._k = key

    def _next(self):
        self._k, sub = jax.random.split(self._k)
        return sub

    def normal(self, shape):
        return jax.random.normal(self._next(), shape, dtype=jnp.bfloat16)

    def randint(self, lo, hi, shape):
        return jax.random.randint(self._next(), shape, lo, hi, dtype=jnp.int32)

    def uniform(self, shape, lo=0.0, hi=1.0):
        return jax.random.uniform(self._next(), shape, jnp.bfloat16, lo, hi)

    def permutation(self, n):
        return jax.random.permutation(self._next(), n)
kernel_name = 'adaLN_cond__sliding_block_cached__glu_gated_bilinear__decode'

def setup_inputs():
    _rng = _Rng(jax.random.key(int.from_bytes(__import__("os").urandom(4), "little")))
    _w = lambda a: (lambda t: t.astype(jnp.bfloat16) if jnp.issubdtype(t.dtype, jnp.floating) else t)(jnp.asarray(a))

    def _A_setup():
        B, Sq, D = (1, 1, 640)
        Hq, Hkv, Sk, Dh = (32, 32, 32768, 192)
        assert Hq % Hkv == 0, (Hq, Hkv)
        return {'x': _w((lambda *s: _rng.normal(s) * 0.05)(B, Sq, D)), 'k_cache': _w((lambda *s: _rng.normal(s) * 0.05)(B, Hkv, Sk, Dh)), 'v_cache': _w((lambda *s: _rng.normal(s) * 0.05)(B, Hkv, Sk, Dh)), 'wq': _w((lambda *s: _rng.normal(s) * 0.05)(D, Hq * Dh) * D ** (-0.5)), 'wo': _w((lambda *s: _rng.normal(s) * 0.05)(Hq * Dh, D) * (Hq * Dh) ** (-0.5))}
    _A_in = _A_setup()

    def _B_setup():
        B, S, D, F = (1, 1, 640, 1536)
        return {'x': _w((lambda *s: _rng.normal(s) * 0.05)(B, S, D)), 'w_gate': _w((lambda *s: _rng.normal(s) * 0.05)(D, F) * D ** (-0.5)), 'w_up': _w((lambda *s: _rng.normal(s) * 0.05)(D, F) * D ** (-0.5)), 'w_down': _w((lambda *s: _rng.normal(s) * 0.05)(F, D) * F ** (-0.5))}
    _B_in = _B_setup()
    return {'A_x': _A_in['x'], 'A_k_cache': _A_in['k_cache'], 'A_v_cache': _A_in['v_cache'], 'A_wq': _A_in['wq'], 'A_wo': _A_in['wo'], 'B_x': _B_in['x'], 'B_w_gate': _B_in['w_gate'], 'B_w_up': _B_in['w_up'], 'B_w_down': _B_in['w_down'], 'c': _w((lambda *s: _rng.normal(s) * 0.05)(1, 640)), 'w_mod': _w((lambda *s: _rng.normal(s) * 0.05)(640, 6 * 640) * 640 ** (-0.5))}

def reference(A_x, A_k_cache, A_v_cache, A_wq, A_wo, B_x, B_w_gate, B_w_up, B_w_down, c, w_mod):

    def _A_ref(x, k_cache, v_cache, wq, wo):
        B, Sq, D = x.shape
        Hq, Dh = (32, 192)
        Hkv, Sk = (k_cache.shape[1], k_cache.shape[2])
        W = min(4096, max(256, Sk // 4))
        rep = Hq // Hkv
        q = (lambda x, *d: x.transpose(*d))((x @ wq).reshape(B, Sq, Hq, Dh), 0, 2, 1, 3)
        k = jnp.repeat(k_cache[:, :, Sk - W:, :], rep, axis=1)
        v = jnp.repeat(v_cache[:, :, Sk - W:, :], rep, axis=1)
        scores = jnp.einsum('bhqd,bhkd->bhqk', q, k) * Dh ** (-0.5)
        p = _softmax(scores, axis=-1)
        o = jnp.einsum('bhqk,bhkd->bhqd', p, v)
        return (lambda x, *d: x.transpose(*d))(o, 0, 2, 1, 3).reshape(B, Sq, Hq * Dh) @ wo

    def _B_ref(x, w_gate, w_up, w_down):
        g = jnp.einsum('bsd,df->bsf', x, w_gate)
        u = jnp.einsum('bsd,df->bsf', x, w_up)
        h = g * u
        return jnp.einsum('bsf,fd->bsd', h, w_down)
    x = A_x
    mod = (_silu(c) @ w_mod).reshape(c.shape[0], 6, 1, -1)
    sa, ca, ga, sb, cb, gb = (mod[:, 0].copy(), mod[:, 1].copy(), mod[:, 2].copy(), mod[:, 3].copy(), mod[:, 4].copy(), mod[:, 5].copy())
    h = _layernorm(x, axis=-1) * (1 + ca) + sa
    x = x + ga * _A_ref(h, A_k_cache, A_v_cache, A_wq, A_wo)
    h = _layernorm(x, axis=-1) * (1 + cb) + sb
    x = x + gb * _B_ref(h, B_w_gate, B_w_up, B_w_down)
    return x
```

```python
import functools

import jax
import jax.numpy as jnp
from jax import lax
import jax.experimental.pallas as pl
import jax.experimental.pallas.tpu as pltpu

_H = 32
_DH = 192
_EPS = 1e-5
_LANES = 128

_CFG = dict(
    g=2,
    depth=2,
    kv_rows=192,
    w_rows=160,
    m=8,
    fchunks=4,
)


def _interleave(a, b):
    out = []
    for i in range(max(len(a), len(b))):
        if i < len(a):
            out.append(a[i])
        if i < len(b):
            out.append(b[i])
    return out


def _layernorm(x):
    m = jnp.mean(x, axis=-1, keepdims=True)
    d = x - m
    v = jnp.mean(d * d, axis=-1, keepdims=True)
    return d / jnp.sqrt(v + _EPS)


def _kernel(x_hbm, c_hbm, kt_hbm, vt_hbm, wq_hbm, wo_hbm, wg_hbm, wu_hbm, wd_hbm, wm_hbm,
            o_ref,
            x_b, c_b, wm_b, k_b, v_b, wq_b, wo_b, wg_b, wu_b, wd_b, h_s, acc_s,
            sem_small, sem_wm, sem_k, sem_v, sem_wq, sem_wo, sem_gu, sem_d,
            *, cfg, d_model, d_ff, sk, win):
    g, depth, m = cfg["g"], cfg["depth"], cfg["m"]
    kv_rows, w_rows, fchunks = cfg["kv_rows"], cfg["w_rows"], cfg["fchunks"]
    gd = g * _DH
    nstage = _H // g
    fc = d_ff // fchunks
    f32, bf16 = jnp.float32, jnp.bfloat16

    def strips(src, dst, sem, r0, nrows, c0, ncols, rows, dr0=0, dc0=0):
        out = []
        for r in range(0, nrows, rows):
            for c in range(0, ncols, _LANES):
                out.append(pltpu.make_async_copy(
                    src.at[pl.ds(r0 + r, rows), pl.ds(c0 + c, _LANES)],
                    dst.at[pl.ds(dr0 + r, rows), pl.ds(dc0 + c, _LANES)],
                    sem))
        return out

    def start_pairs(a, b):
        for cp, p in _interleave([(x, 0) for x in a], [(x, 1) for x in b]):
            cp.start(priority=p)

    def start_split(cps):
        start_pairs(cps[: len(cps) // 2], cps[len(cps) // 2:])

    def wait_all(ref, sem):
        pltpu.make_async_copy(ref, ref, sem).wait()

    def issue_stage(s):
        slot = s % depth
        r0 = pl.multiple_of(s * gd, gd)
        start_pairs(
            strips(wq_hbm, wq_b.at[slot], sem_wq.at[slot], 0, d_model, r0, gd, w_rows),
            strips(wo_hbm, wo_b.at[slot], sem_wo.at[slot], r0, gd, 0, d_model, _DH))
        start_pairs(
            strips(kt_hbm, k_b.at[slot], sem_k.at[slot], r0, gd, sk - win, win, kv_rows),
            strips(vt_hbm, v_b.at[slot], sem_v.at[slot], r0, gd, sk - win, win, kv_rows))

    def issue_tail():
        start_split(strips(wm_hbm, wm_b, sem_wm.at[1], 0, d_model, 2 * d_model, 4 * d_model,
                           w_rows, dc0=2 * d_model))
        for j in range(fchunks):
            start_pairs(
                strips(wg_hbm, wg_b, sem_gu.at[j], 0, d_model, j * fc, fc, w_rows, dc0=j * fc),
                strips(wu_hbm, wu_b, sem_gu.at[j], 0, d_model, j * fc, fc, w_rows, dc0=j * fc))
            start_split(strips(wd_hbm, wd_b, sem_d.at[j], j * fc, fc, 0, d_model, _DH, dr0=j * fc))

    cx = pltpu.make_async_copy(x_hbm, x_b, sem_small.at[0])
    cc = pltpu.make_async_copy(c_hbm, c_b, sem_small.at[1])
    cx.start(priority=0)
    cc.start(priority=1)
    start_split(strips(wm_hbm, wm_b, sem_wm.at[0], 0, d_model, 0, 2 * d_model, w_rows))

    def pro(s, carry):
        issue_stage(s)
        return carry
    lax.fori_loop(0, depth, pro, 0)

    cx.wait()
    cc.wait()
    cv = jnp.broadcast_to(c_b[...].astype(f32), (m, d_model))
    sc = (cv * jax.nn.sigmoid(cv)).astype(bf16)
    x = jnp.broadcast_to(x_b[...].astype(f32), (m, d_model))
    wait_all(wm_b.at[:, pl.ds(0, 2 * d_model)], sem_wm.at[0])
    mod = jnp.dot(sc, wm_b[:, pl.ds(0, 2 * d_model)], preferred_element_type=f32)
    h_s[...] = (_layernorm(x) * (1.0 + mod[:, d_model:]) + mod[:, :d_model]).astype(bf16)
    acc_s[...] = jnp.zeros_like(acc_s)

    row = lax.broadcasted_iota(jnp.int32, (m, gd), 0)
    col = lax.broadcasted_iota(jnp.int32, (m, gd), 1)
    diag = (col >= row * _DH) & (col < (row + 1) * _DH)

    def stage(s, carry):
        slot = s % depth
        wait_all(wq_b.at[slot], sem_wq.at[slot])
        q = jnp.dot(h_s[...], wq_b[slot], preferred_element_type=f32)
        q = jnp.where(diag, q, 0.0).astype(bf16)
        wait_all(k_b.at[slot], sem_k.at[slot])
        sco = jnp.dot(q, k_b[slot], preferred_element_type=f32) * (_DH ** -0.5)
        e = jnp.exp(sco - jnp.max(sco, axis=-1, keepdims=True))
        l = jnp.sum(e, axis=-1, keepdims=True)
        wait_all(v_b.at[slot], sem_v.at[slot])
        o = lax.dot_general(e.astype(bf16), v_b[slot], (((1,), (1,)), ((), ())),
                            preferred_element_type=f32)
        o = jnp.where(diag, o / l, 0.0).astype(bf16)
        wait_all(wo_b.at[slot], sem_wo.at[slot])
        acc_s[...] += jnp.dot(o, wo_b[slot], preferred_element_type=f32)

        @pl.when(s + depth < nstage)
        def _():
            issue_stage(s + depth)

        @pl.when(s + depth == nstage - 1)
        def _():
            issue_tail()
        return carry
    lax.fori_loop(0, nstage, stage, 0)

    attn = jnp.sum(acc_s[...], axis=0, keepdims=True)
    wait_all(wm_b.at[:, pl.ds(2 * d_model, 4 * d_model)], sem_wm.at[1])
    mod = jnp.dot(sc, wm_b[:, pl.ds(2 * d_model, 4 * d_model)], preferred_element_type=f32)
    ga, sb = mod[:, :d_model], mod[:, d_model:2 * d_model]
    cb, gb = mod[:, 2 * d_model:3 * d_model], mod[:, 3 * d_model:]
    x1 = x + ga * attn
    h2 = (_layernorm(x1) * (1.0 + cb) + sb).astype(bf16)
    y = jnp.zeros((m, d_model), f32)
    for j in range(fchunks):
        wait_all(wg_b.at[:, pl.ds(j * fc, fc)], sem_gu.at[j])
        wait_all(wu_b.at[:, pl.ds(j * fc, fc)], sem_gu.at[j])
        gg = jnp.dot(h2, wg_b[:, pl.ds(j * fc, fc)], preferred_element_type=f32)
        uu = jnp.dot(h2, wu_b[:, pl.ds(j * fc, fc)], preferred_element_type=f32)
        hh = (gg * uu).astype(bf16)
        wait_all(wd_b.at[pl.ds(j * fc, fc), :], sem_d.at[j])
        y = y + jnp.dot(hh, wd_b[pl.ds(j * fc, fc), :], preferred_element_type=f32)
    out = x1 + gb * y
    o_ref[...] = out[0:1, :].astype(o_ref.dtype)


def _build(cfg, A_x, A_k_cache, A_v_cache, A_wq, A_wo, B_w_gate, B_w_up, B_w_down, c, w_mod):
    b, sq, d_model = A_x.shape
    _, hkv, sk, dh = A_k_cache.shape
    assert b == 1 and sq == 1 and hkv == _H and dh == _DH
    d_ff = B_w_gate.shape[1]
    win = min(4096, max(256, sk // 4))
    g, depth, m, fchunks = cfg["g"], cfg["depth"], cfg["m"], cfg["fchunks"]
    gd = g * _DH
    bf16 = jnp.bfloat16

    kt = jnp.transpose(A_k_cache, (0, 1, 3, 2)).reshape(_H * _DH, sk)
    vt = jnp.transpose(A_v_cache, (0, 1, 3, 2)).reshape(_H * _DH, sk)
    x2 = A_x.reshape(1, d_model)

    kern = functools.partial(_kernel, cfg=cfg, d_model=d_model, d_ff=d_ff, sk=sk, win=win)
    dma = pltpu.SemaphoreType.DMA
    out = pl.pallas_call(
        kern,
        out_shape=jax.ShapeDtypeStruct((1, d_model), A_x.dtype),
        in_specs=[pl.BlockSpec(memory_space=pl.ANY)] * 10,
        out_specs=pl.BlockSpec(memory_space=pltpu.VMEM),
        scratch_shapes=[
            pltpu.VMEM((1, d_model), bf16),
            pltpu.VMEM((1, d_model), bf16),
            pltpu.VMEM((d_model, 6 * d_model), bf16),
            pltpu.VMEM((depth, gd, win), bf16),
            pltpu.VMEM((depth, gd, win), bf16),
            pltpu.VMEM((depth, d_model, gd), bf16),
            pltpu.VMEM((depth, gd, d_model), bf16),
            pltpu.VMEM((d_model, d_ff), bf16),
            pltpu.VMEM((d_model, d_ff), bf16),
            pltpu.VMEM((d_ff, d_model), bf16),
            pltpu.VMEM((m, d_model), bf16),
            pltpu.VMEM((m, d_model), jnp.float32),
            dma((2,)), dma((2,)), dma((depth,)), dma((depth,)), dma((depth,)), dma((depth,)),
            dma((fchunks,)), dma((fchunks,)),
        ],
        compiler_params=pltpu.CompilerParams(vmem_limit_bytes=100 * 1024 * 1024),
    )(x2, c, kt, vt, A_wq, A_wo, B_w_gate, B_w_up, B_w_down, w_mod)
    return out.reshape(1, 1, d_model)


@jax.jit
def pallas_adaLN_cond__sliding_block_cached__glu_gated_bilinear__decode_kernel(
    A_x: jax.Array,
    A_k_cache: jax.Array,
    A_v_cache: jax.Array,
    A_wq: jax.Array,
    A_wo: jax.Array,
    B_x: jax.Array,
    B_w_gate: jax.Array,
    B_w_up: jax.Array,
    B_w_down: jax.Array,
    c: jax.Array,
    w_mod: jax.Array,
):
    del B_x
    return _build(_CFG, A_x, A_k_cache, A_v_cache, A_wq, A_wo, B_w_gate, B_w_up, B_w_down, c, w_mod)
```

```python
import functools

import jax
import jax.numpy as jnp
from jax import lax
import jax.experimental.pallas as pl
import jax.experimental.pallas.tpu as pltpu

_H = 32
_DH = 192
_EPS = 1e-5

_CFG = dict(
    g=2, nb=4, la=3, m=8,
    kv=(192, 128), kv_colmajor=False,
    wq=(160, 128), wo=(32, 640), wm=(160, 128), wgu=(160, 128), wd=(32, 640),
    nwm=3,
    fch=4,
    wfirst=True,
)


def _layernorm(x):
    m = jnp.mean(x, axis=-1, keepdims=True)
    d = x - m
    v = jnp.mean(d * d, axis=-1, keepdims=True)
    return d / jnp.sqrt(v + _EPS)


def _kernel(x_hbm, c_hbm, kt_hbm, vt_hbm, wq_hbm, wo_hbm, wg_hbm, wu_hbm, wd_hbm, wm_hbm,
            o_ref,
            x_b, c_b, wm_b, k_b, v_b, wq_b, wo_b, wg_b, wu_b, wd_b, h_s, acc_s, mod_s,
            sems,
            *, cfg, d_model, d_ff, sk, win):
    g, m, nb, la = cfg["g"], cfg["m"], cfg["nb"], cfg["la"]
    fch, nwm = cfg["fch"], cfg["nwm"]
    gd = g * _DH
    nstage = _H // g
    fc = d_ff // fch
    cw = win // nb
    f32, bf16 = jnp.float32, jnp.bfloat16
    nocompute = cfg.get("nocompute", False)

    S_X, S_C = 0, 1
    S_WM = 2
    S_K = S_WM + nwm
    S_V = S_K + nb
    S_WQ = S_V + nb
    S_WO = S_WQ + 2
    S_G = S_WO + 2
    S_U = S_G + fch
    S_D = S_U + fch

    def pieces(src, dst, sem, r0, nrows, c0, ncols, shp, dr0=0, dc0=0, colmajor=False):
        rows, cols = min(shp[0], nrows), min(shp[1], ncols)
        assert nrows % rows == 0 and ncols % cols == 0, (nrows, ncols, shp)
        if colmajor:
            idx = [(r, c) for c in range(0, ncols, cols) for r in range(0, nrows, rows)]
        else:
            idx = [(r, c) for r in range(0, nrows, rows) for c in range(0, ncols, cols)]
        return [pltpu.make_async_copy(
            src.at[pl.ds(r0 + r, rows), pl.ds(c0 + c, cols)],
            dst.at[pl.ds(dr0 + r, rows), pl.ds(dc0 + c, cols)],
            sems.at[sem]) for r, c in idx]

    def start_pairs(a, b):
        i = j = 0
        while i < len(a) or j < len(b):
            if j >= len(b) or (i < len(a) and i * len(b) <= j * len(a)):
                a[i].start(priority=0)
                i += 1
            else:
                b[j].start(priority=1)
                j += 1

    def start_split(cps):
        start_pairs(cps[: len(cps) // 2], cps[len(cps) // 2:])

    def wait_all(ref, sem):
        pltpu.make_async_copy(ref, ref, sems.at[sem]).wait()

    wmc = 6 * d_model // nwm

    def issue_wm(j):
        start_split(pieces(wm_hbm, wm_b, S_WM + j, 0, d_model, j * wmc, wmc, cfg["wm"], dc0=j * wmc))

    def issue_kv(s, j):
        slot = s % 2
        r0 = pl.multiple_of(s * gd, gd)
        qr, orr = d_model // nb, gd // nb
        a = pieces(wq_hbm, wq_b.at[slot], S_WQ + slot, j * qr, qr, r0, gd, cfg["wq"], dr0=j * qr)
        b = pieces(wo_hbm, wo_b.at[slot], S_WO + slot, r0 + j * orr, orr, 0, d_model, cfg["wo"], dr0=j * orr)
        ka = pieces(kt_hbm, k_b.at[slot], S_K + j, r0, gd, sk - win + j * cw, cw, cfg["kv"], dc0=j * cw,
                    colmajor=cfg["kv_colmajor"])
        vb = pieces(vt_hbm, v_b.at[slot], S_V + j, r0, gd, sk - win + j * cw, cw, cfg["kv"], dc0=j * cw,
                    colmajor=cfg["kv_colmajor"])
        if cfg["wfirst"]:
            start_pairs(a, b)
            start_pairs(ka, vb)
        else:
            start_pairs(ka, vb)
            start_pairs(a, b)

    def issue_ffn(j):
        start_pairs(
            pieces(wg_hbm, wg_b, S_G + j, 0, d_model, j * fc, fc, cfg["wgu"], dc0=j * fc),
            pieces(wu_hbm, wu_b, S_U + j, 0, d_model, j * fc, fc, cfg["wgu"], dc0=j * fc))
        start_split(pieces(wd_hbm, wd_b, S_D + j, j * fc, fc, 0, d_model, cfg["wd"], dr0=j * fc))

    cx = pltpu.make_async_copy(x_hbm, x_b, sems.at[S_X])
    cc = pltpu.make_async_copy(c_hbm, c_b, sems.at[S_C])
    cx.start(priority=0)
    cc.start(priority=1)
    pro = [functools.partial(issue_wm, j) for j in range(nwm)] + \
          [functools.partial(issue_kv, 0, j) for j in range(la)]
    for t in range(la):
        pro[t]()
    cx.wait()
    cc.wait()
    cv = jnp.broadcast_to(c_b[...].astype(f32), (m, d_model))
    sc = (cv * jax.nn.sigmoid(cv)).astype(bf16)
    for j in range(nwm):
        wait_all(wm_b.at[:, pl.ds(j * wmc, wmc)], S_WM + j)
        pro[j + la]()
        mod_s[:, pl.ds(j * wmc, wmc)] = jnp.dot(sc, wm_b[:, pl.ds(j * wmc, wmc)], preferred_element_type=f32)
    x = jnp.broadcast_to(x_b[...].astype(f32), (m, d_model))
    h_s[...] = (_layernorm(x) * (1.0 + mod_s[:, pl.ds(d_model, d_model)]) + mod_s[:, pl.ds(0, d_model)]).astype(bf16)
    acc_s[...] = jnp.zeros_like(acc_s)

    def stage(s, carry):
        slot = s % 2
        for j in range(nb):
            wait_all(k_b.at[slot, :, pl.ds(j * cw, cw)], S_K + j)
            wait_all(v_b.at[slot, :, pl.ds(j * cw, cw)], S_V + j)
            if j + la < nb:
                issue_kv(s, j + la)
            else:
                @pl.when(s + 1 < nstage)
                def _():
                    issue_kv(s + 1, j + la - nb)

                @pl.when(s + 1 == nstage)
                def _():
                    issue_ffn(j + la - nb)
        wait_all(wq_b.at[slot], S_WQ + slot)
        wait_all(wo_b.at[slot], S_WO + slot)
        if nocompute:
            return carry
        row = lax.broadcasted_iota(jnp.int32, (m, gd), 0)
        col = lax.broadcasted_iota(jnp.int32, (m, gd), 1)
        diag = (col >= row * _DH) & (col < (row + 1) * _DH)
        q = jnp.dot(h_s[...], wq_b[slot], preferred_element_type=f32)
        q = jnp.where(diag, q, 0.0).astype(bf16)
        sco = jnp.dot(q, k_b[slot], preferred_element_type=f32) * (_DH ** -0.5)
        e = jnp.exp(sco - jnp.max(sco, axis=-1, keepdims=True))
        l = jnp.sum(e, axis=-1, keepdims=True)
        o = lax.dot_general(e.astype(bf16), v_b[slot], (((1,), (1,)), ((), ())),
                            preferred_element_type=f32)
        o = jnp.where(diag, o / l, 0.0).astype(bf16)
        acc_s[...] += jnp.dot(o, wo_b[slot], preferred_element_type=f32)
        return carry
    lax.fori_loop(0, nstage, stage, 0)

    attn = jnp.sum(acc_s[...], axis=0, keepdims=True)
    x = jnp.broadcast_to(x_b[...].astype(f32), (m, d_model))
    x1 = x + mod_s[:, pl.ds(2 * d_model, d_model)] * attn
    h2 = (_layernorm(x1) * (1.0 + mod_s[:, pl.ds(4 * d_model, d_model)])
          + mod_s[:, pl.ds(3 * d_model, d_model)]).astype(bf16)
    y = jnp.zeros((m, d_model), f32)
    for j in range(fch):
        wait_all(wg_b.at[:, pl.ds(j * fc, fc)], S_G + j)
        wait_all(wu_b.at[:, pl.ds(j * fc, fc)], S_U + j)
        if j + la < fch:
            issue_ffn(j + la)
        gg = jnp.dot(h2, wg_b[:, pl.ds(j * fc, fc)], preferred_element_type=f32)
        uu = jnp.dot(h2, wu_b[:, pl.ds(j * fc, fc)], preferred_element_type=f32)
        hh = (gg * uu).astype(bf16)
        wait_all(wd_b.at[pl.ds(j * fc, fc), :], S_D + j)
        y = y + jnp.dot(hh, wd_b[pl.ds(j * fc, fc), :], preferred_element_type=f32)
    out = x1 + mod_s[:, pl.ds(5 * d_model, d_model)] * y
    o_ref[...] = out[0:1, :].astype(o_ref.dtype)


def _build(cfg, A_x, A_k_cache, A_v_cache, A_wq, A_wo, B_w_gate, B_w_up, B_w_down, c, w_mod):
    b, sq, d_model = A_x.shape
    _, hkv, sk, dh = A_k_cache.shape
    d_ff = B_w_gate.shape[1]
    win = min(4096, max(256, sk // 4))
    g, m = cfg["g"], cfg["m"]
    gd = g * _DH
    bf16 = jnp.bfloat16
    kt = jnp.transpose(A_k_cache, (0, 1, 3, 2)).reshape(_H * _DH, sk)
    vt = jnp.transpose(A_v_cache, (0, 1, 3, 2)).reshape(_H * _DH, sk)
    x2 = A_x.reshape(1, d_model)
    kern = functools.partial(_kernel, cfg=cfg, d_model=d_model, d_ff=d_ff, sk=sk, win=win)
    nsem = 2 + cfg["nwm"] + 2 * cfg["nb"] + 4 + 3 * cfg["fch"]
    out = pl.pallas_call(
        kern,
        out_shape=jax.ShapeDtypeStruct((1, d_model), A_x.dtype),
        in_specs=[pl.BlockSpec(memory_space=pl.ANY)] * 10,
        out_specs=pl.BlockSpec(memory_space=pltpu.VMEM),
        scratch_shapes=[
            pltpu.VMEM((1, d_model), bf16),
            pltpu.VMEM((1, d_model), bf16),
            pltpu.VMEM((d_model, 6 * d_model), bf16),
            pltpu.VMEM((2, gd, win), bf16),
            pltpu.VMEM((2, gd, win), bf16),
            pltpu.VMEM((2, d_model, gd), bf16),
            pltpu.VMEM((2, gd, d_model), bf16),
            pltpu.VMEM((d_model, d_ff), bf16),
            pltpu.VMEM((d_model, d_ff), bf16),
            pltpu.VMEM((d_ff, d_model), bf16),
            pltpu.VMEM((m, d_model), bf16),
            pltpu.VMEM((m, d_model), jnp.float32),
            pltpu.VMEM((m, 6 * d_model), jnp.float32),
            pltpu.SemaphoreType.DMA((nsem,)),
        ],
        compiler_params=pltpu.CompilerParams(vmem_limit_bytes=100 * 1024 * 1024,
                                             disable_bounds_checks=True,
                                             disable_semaphore_checks=True),
    )(x2, c, kt, vt, A_wq, A_wo, B_w_gate, B_w_up, B_w_down, w_mod)
    return out.reshape(1, 1, d_model)


@jax.jit
def pallas_adaLN_cond__sliding_block_cached__glu_gated_bilinear__decode_kernel(
    A_x: jax.Array,
    A_k_cache: jax.Array,
    A_v_cache: jax.Array,
    A_wq: jax.Array,
    A_wo: jax.Array,
    B_x: jax.Array,
    B_w_gate: jax.Array,
    B_w_up: jax.Array,
    B_w_down: jax.Array,
    c: jax.Array,
    w_mod: jax.Array,
):
    del B_x
    return _build(_CFG, A_x, A_k_cache, A_v_cache, A_wq, A_wo, B_w_gate, B_w_up, B_w_down, c, w_mod)
```

```python
import functools

import jax
import jax.numpy as jnp
from jax import lax
import jax.experimental.pallas as pl
import jax.experimental.pallas.tpu as pltpu

_H = 32
_DH = 192
_EPS = 1e-5

_CFG = dict(
    m=8, nvb=4, dsplit=(384, 384, 384, 384),
    kv=(192, 128), kb=1, vb=1,
    wq=(8, 768), wo=(8, 640), wg=(8, 768), wm=(8, 768), wu=(8, 1536), wd=(48, 640),
    na=5,
    wu_split=(192, 192),
    lfirst=0,
)


def _layernorm(x):
    m = jnp.mean(x, axis=-1, keepdims=True)
    d = x - m
    v = jnp.mean(d * d, axis=-1, keepdims=True)
    return d / jnp.sqrt(v + _EPS)


def _merge(*lists):
    items = []
    for li, l in enumerate(lists):
        for i, x in enumerate(l):
            items.append(((i + 0.5) / len(l), li, i, x))
    items.sort(key=lambda t: t[:3])
    return [t[3] for t in items]


def _kernel(x_hbm, c_hbm, kt_hbm, vt_hbm, wq_hbm, wo_hbm, wg_hbm, wu_hbm, wd_hbm, wm_hbm,
            o_ref,
            x_b, c_b, wm_b, k_b, v_b, wq_b, wo_b, wg_b, wu_b, wd_b, mod_s, q_s, acc_s, e_s, l_s,
            sems,
            *, cfg, d_model, d_ff, sk, win):
    m, nvb, dsplit = cfg["m"], cfg["nvb"], cfg["dsplit"]
    ndch = len(dsplit)
    assert sum(dsplit) == d_ff
    gd = 2 * _DH
    nstage = _H // 2
    last = nstage - 1
    cw = win // nvb
    er = d_model // nstage
    na = cfg["na"]
    nbu = last - na
    f32, bf16 = jnp.float32, jnp.bfloat16
    nocompute = cfg.get("nocompute", False)

    S_X, S_C, S_WM, S_WQ, S_G, S_U, S_V0 = range(7)
    S_K, S_WO = 7, 9
    S_V = 11
    S_D = S_V + nvb

    def pieces(src, dst, sem, r0, nrows, c0, ncols, shp, dr0=0, dc0=0):
        if nrows == 0:
            return []
        rows, cols = min(shp[0], nrows), min(shp[1], ncols)
        assert nrows % rows == 0 and ncols % cols == 0, (nrows, ncols, shp)
        return [pltpu.make_async_copy(
            src.at[pl.ds(r0 + r, rows), pl.ds(c0 + c, cols)],
            dst.at[pl.ds(dr0 + r, rows), pl.ds(dc0 + c, cols)],
            sems.at[sem]) for r in range(0, nrows, rows) for c in range(0, ncols, cols)]

    def start_unit(ls, hs, lfirst=0):
        for cp in ls[:lfirst]:
            cp.start(priority=1)
        for cp, p in _merge([(x, 1) for x in ls[lfirst:]], [(x, 0) for x in hs]):
            cp.start(priority=p)

    def wait_all(ref, sem):
        pltpu.make_async_copy(ref, ref, sems.at[sem]).wait()

    def al(v, k):
        return v if isinstance(v, int) else pl.multiple_of(v, k)

    def kv_strips(src, dst, s, nb, sem_of):
        r0 = al(s * gd, gd)
        w = win // nb
        out = []
        for j in range(nb):
            out += pieces(src, dst, sem_of(j), r0, gd, sk - win + j * w, w, cfg["kv"], dc0=j * w)
        return out

    def half(lst, h):
        n = len(lst) // 2
        for cp in (lst[n:] if h == 0 else lst[:n]):
            cp._used = True
        return lst[:n] if h == 0 else lst[n:]

    def rows_of(src, dst, sem, r0, nrows, shp):
        return pieces(src, dst, sem, r0, nrows, 0, src.shape[1], shp, dr0=r0)

    def k_half(s, h):
        ls = half(kv_strips(kt_hbm, k_b.at[s % 2], s, cfg["kb"], lambda j: S_K + s % 2), h)
        wo = pieces(wo_hbm, wo_b.at[s], S_WO + s % 2, al(s * gd + h * _DH, _DH), _DH, 0, d_model,
                    cfg["wo"], dr0=h * _DH)
        wg = half(rows_of(wg_hbm, wg_b, S_G, al(s * er, er), er, cfg["wg"]), h)
        start_unit(ls, _merge(wo, wg))

    u0, u1 = cfg["wu_split"]

    def v15_half(h):
        ls = half(kv_strips(vt_hbm, v_b.at[last], last, nvb, lambda j: S_V + j), h)
        start_unit(ls, rows_of(wu_hbm, wu_b, S_U, h * u0, (u0, u1)[h], cfg["wu"]))

    def tail():
        ds, r = [], 0
        for j in range(ndch):
            ds += rows_of(wd_hbm, wd_b, S_D + j, r, dsplit[j], cfg["wd"])
            r += dsplit[j]
        start_unit(ds, rows_of(wu_hbm, wu_b, S_U, u0 + u1, d_model - u0 - u1, cfg["wu"]))

    cx = pltpu.make_async_copy(x_hbm, x_b, sems.at[S_X])
    cc = pltpu.make_async_copy(c_hbm, c_b, sems.at[S_C])
    ra, rb = d_model // na, d_model // nbu

    def unit_a(u, lfirst=0):
        start_unit(kv_strips(vt_hbm, v_b.at[u], u, cfg["vb"], lambda j: S_V0),
                   rows_of(wm_hbm, wm_b, S_WM, al(u * ra, ra), ra, cfg["wm"]), lfirst=lfirst)

    def unit_b(u):
        start_unit(kv_strips(vt_hbm, v_b.at[u], u, cfg["vb"], lambda j: S_V0),
                   rows_of(wq_hbm, wq_b, S_WQ, al((u - na) * rb, rb), rb, cfg["wq"]))

    if cfg["lfirst"]:
        unit_a(0, cfg["lfirst"])
        cx.start(priority=0)
        cc.start(priority=0)
        lax.fori_loop(1, na, lambda u, c: (unit_a(u), c)[1], 0)
    else:
        cx.start(priority=0)
        cc.start(priority=0)
        lax.fori_loop(0, na, lambda u, c: (unit_a(u), c)[1], 0)

    def phase_b(u, carry):
        unit_b(u)

        @pl.when(u == na)
        def _():
            cc.wait()
            cv = jnp.broadcast_to(c_b[...].astype(f32), (m, d_model))
            sc = (cv * jax.nn.sigmoid(cv)).astype(bf16)
            wait_all(wm_b, S_WM)
            mod_s[...] = jnp.dot(sc, wm_b[...], preferred_element_type=f32)
        return carry
    lax.fori_loop(na, last, phase_b, 0)

    k_half(0, 0)
    cx.wait()
    x = jnp.broadcast_to(x_b[...].astype(f32), (m, d_model))
    h = (_layernorm(x) * (1.0 + mod_s[:, pl.ds(d_model, d_model)]) + mod_s[:, pl.ds(0, d_model)]).astype(bf16)
    row = lax.broadcasted_iota(jnp.int32, (m, gd), 0)
    col = lax.broadcasted_iota(jnp.int32, (m, gd), 1)
    diag = (col >= row * _DH) & (col < (row + 1) * _DH)
    wait_all(wq_b, S_WQ)
    q = jnp.dot(h, wq_b[...], preferred_element_type=f32)
    for s in range(nstage):
        q_s[s] = jnp.where(diag, q[:, s * gd:(s + 1) * gd], 0.0).astype(bf16)
    acc_s[...] = jnp.zeros_like(acc_s)
    k_half(0, 1)
    k_half(1, 0)
    wait_all(v_b.at[pl.ds(0, last)], S_V0)

    def stage(s, carry):
        slot = s % 2

        @pl.when(s < last)
        def _():
            k_half(s + 1, 1)

        @pl.when(s == last)
        def _():
            v15_half(1)

        wait_all(k_b.at[slot], S_K + slot)
        wait_all(wo_b.at[s], S_WO + slot)
        if not nocompute:
            sco = jnp.dot(q_s[s], k_b[slot], preferred_element_type=f32) * (_DH ** -0.5)
            e = jnp.exp(sco - jnp.max(sco, axis=-1, keepdims=True))
            l_s[...] = jnp.broadcast_to(jnp.sum(e, axis=-1, keepdims=True), l_s.shape)
            e_s[...] = e.astype(bf16)

        @pl.when(s < last - 1)
        def _():
            k_half(s + 2, 0)

        @pl.when(s == last - 1)
        def _():
            v15_half(0)

        @pl.when(s == last)
        def _():
            tail()

        o = jnp.zeros((m, gd), f32)
        for j in range(nvb):
            @pl.when(s == last)
            def _():
                wait_all(v_b.at[last, :, pl.ds(j * cw, cw)], S_V + j)
            if not nocompute:
                o = o + lax.dot_general(e_s[:, pl.ds(j * cw, cw)], v_b[s, :, pl.ds(j * cw, cw)],
                                        (((1,), (1,)), ((), ())), preferred_element_type=f32)
        if not nocompute:
            row = lax.broadcasted_iota(jnp.int32, (m, gd), 0)
            col = lax.broadcasted_iota(jnp.int32, (m, gd), 1)
            diag = (col >= row * _DH) & (col < (row + 1) * _DH)
            o = jnp.where(diag, o / l_s[:, 0:1], 0.0).astype(bf16)
            acc_s[...] += jnp.dot(o, wo_b[s], preferred_element_type=f32)
        return carry
    lax.fori_loop(0, nstage, stage, 0)

    attn = jnp.sum(acc_s[...], axis=0, keepdims=True)
    x = jnp.broadcast_to(x_b[...].astype(f32), (m, d_model))
    x1 = x + mod_s[:, pl.ds(2 * d_model, d_model)] * attn
    h2 = (_layernorm(x1) * (1.0 + mod_s[:, pl.ds(4 * d_model, d_model)])
          + mod_s[:, pl.ds(3 * d_model, d_model)]).astype(bf16)
    wait_all(wg_b, S_G)
    wait_all(wu_b, S_U)
    gg = jnp.dot(h2, wg_b[...], preferred_element_type=f32)
    uu = jnp.dot(h2, wu_b[...], preferred_element_type=f32)
    hh = (gg * uu).astype(bf16)
    y = jnp.zeros((m, d_model), f32)
    r = 0
    for j in range(ndch):
        wait_all(wd_b.at[pl.ds(r, dsplit[j]), :], S_D + j)
        y = y + jnp.dot(hh[:, r:r + dsplit[j]], wd_b[pl.ds(r, dsplit[j]), :], preferred_element_type=f32)
        r += dsplit[j]
    out = x1 + mod_s[:, pl.ds(5 * d_model, d_model)] * y
    o_ref[...] = out[0:1, :].astype(o_ref.dtype)


def _build(cfg, A_x, A_k_cache, A_v_cache, A_wq, A_wo, B_w_gate, B_w_up, B_w_down, c, w_mod):
    b, sq, d_model = A_x.shape
    _, hkv, sk, dh = A_k_cache.shape
    d_ff = B_w_gate.shape[1]
    win = min(4096, max(256, sk // 4))
    m = cfg["m"]
    gd = 2 * _DH
    nstage = _H // 2
    bf16 = jnp.bfloat16
    kt = jnp.transpose(A_k_cache, (0, 1, 3, 2)).reshape(_H * _DH, sk)
    vt = jnp.transpose(A_v_cache, (0, 1, 3, 2)).reshape(_H * _DH, sk)
    x2 = A_x.reshape(1, d_model)
    kern = functools.partial(_kernel, cfg=cfg, d_model=d_model, d_ff=d_ff, sk=sk, win=win)
    nsem = 11 + cfg["nvb"] + len(cfg["dsplit"])
    out = pl.pallas_call(
        kern,
        out_shape=jax.ShapeDtypeStruct((1, d_model), A_x.dtype),
        in_specs=[pl.BlockSpec(memory_space=pl.ANY)] * 10,
        out_specs=pl.BlockSpec(memory_space=pltpu.VMEM),
        scratch_shapes=[
            pltpu.VMEM((1, d_model), bf16),
            pltpu.VMEM((1, d_model), bf16),
            pltpu.VMEM((d_model, 6 * d_model), bf16),
            pltpu.VMEM((2, gd, win), bf16),
            pltpu.VMEM((nstage, gd, win), bf16),
            pltpu.VMEM((d_model, _H * _DH), bf16),
            pltpu.VMEM((nstage, gd, d_model), bf16),
            pltpu.VMEM((d_model, d_ff), bf16),
            pltpu.VMEM((d_model, d_ff), bf16),
            pltpu.VMEM((d_ff, d_model), bf16),
            pltpu.VMEM((m, 6 * d_model), jnp.float32),
            pltpu.VMEM((nstage, m, gd), bf16),
            pltpu.VMEM((m, d_model), jnp.float32),
            pltpu.VMEM((m, win), bf16),
            pltpu.VMEM((m, 128), jnp.float32),
            pltpu.SemaphoreType.DMA((nsem,)),
        ],
        compiler_params=pltpu.CompilerParams(vmem_limit_bytes=110 * 1024 * 1024,
                                             disable_bounds_checks=True,
                                             disable_semaphore_checks=True),
    )(x2, c, kt, vt, A_wq, A_wo, B_w_gate, B_w_up, B_w_down, w_mod)
    return out.reshape(1, 1, d_model)


@jax.jit
def pallas_adaLN_cond__sliding_block_cached__glu_gated_bilinear__decode_kernel(
    A_x: jax.Array,
    A_k_cache: jax.Array,
    A_v_cache: jax.Array,
    A_wq: jax.Array,
    A_wo: jax.Array,
    B_x: jax.Array,
    B_w_gate: jax.Array,
    B_w_up: jax.Array,
    B_w_down: jax.Array,
    c: jax.Array,
    w_mod: jax.Array,
):
    del B_x
    return _build(_CFG, A_x, A_k_cache, A_v_cache, A_wq, A_wo, B_w_gate, B_w_up, B_w_down, c, w_mod)
```

```python
import functools

import jax
import jax.numpy as jnp
from jax import lax
import jax.experimental.pallas as pl
import jax.experimental.pallas.tpu as pltpu

_H = 32
_DH = 192
_GD = 2 * _DH
_NS = _H // 2
_EPS = 1e-5
_M = 8
_HI, _LO = 0, 1

_CFG = dict(
    nvb=4,
    dsplit=(896, 384, 128, 128),
    kv=(192, 128),
    wm=(8, 768), wq=(8, 768), wo=(8, 640), wgu=(8, 768), wd=(64, 640),
    na=5,
    wu_k=24,
    wu_v=(88, 88),
)


def _layernorm(x):
    m = jnp.mean(x, axis=-1, keepdims=True)
    d = x - m
    v = jnp.mean(d * d, axis=-1, keepdims=True)
    return d / jnp.sqrt(v + _EPS)


def _merge(*lists):
    items = []
    for li, lst in enumerate(lists):
        for i, x in enumerate(lst):
            items.append(((i + 0.5) / len(lst), li, i, x))
    items.sort(key=lambda t: t[:3])
    return [t[3] for t in items]


def _half(lst, h):
    n = len(lst) // 2
    return lst[:n] if h == 0 else lst[n:]


def _al(v, k):
    return v if isinstance(v, int) else pl.multiple_of(v, k)


def _diag():
    row = lax.broadcasted_iota(jnp.int32, (_M, _GD), 0)
    col = lax.broadcasted_iota(jnp.int32, (_M, _GD), 1)
    return (col >= row * _DH) & (col < (row + 1) * _DH)


def _kernel(x_hbm, c_hbm, kt_hbm, vt_hbm, wq_hbm, wo_hbm, wg_hbm, wu_hbm, wd_hbm, wm_hbm,
            o_ref,
            x_b, c_b, wm_b, k_b, v_b, wq_b, wo_b, wg_b, wu_b, wd_b,
            mod_s, q_s, acc_s, e_s, l_s, o_s, hb_s,
            sems,
            *, cfg, d_model, d_ff, sk, win):
    f32, bf16 = jnp.float32, jnp.bfloat16
    nvb, dsplit, na = cfg["nvb"], cfg["dsplit"], cfg["na"]
    last = _NS - 1
    cw = win // nvb
    w0 = sk - win
    ra, rb, rg = d_model // na, d_model // (last - na), d_model // _NS
    uk = cfg["wu_k"]
    u0, u1 = cfg["wu_v"]
    ub = uk * _NS
    vr = dsplit[-1]
    assert sum(dsplit) == d_ff and vr == 128

    s_x, s_c, s_wm, s_wq, s_g, s_u, s_v0, s_k, s_wo, s_v = 0, 1, 2, 3, 4, 5, 6, 7, 9, 11
    s_d = s_v + nvb

    def pieces(src, dst, sem, r0, nrows, c0, ncols, shp, dr0, dc0):
        rows, cols = shp
        assert nrows % rows == 0 and ncols % cols == 0, (nrows, ncols, shp)
        return [(src, r0, c0, dst, dr0, dc0, r, c, rows, cols, sem)
                for r in range(0, nrows, rows) for c in range(0, ncols, cols)]

    def rows_of(src, dst, sem, r0, nrows, shp):
        return pieces(src, dst, sem, r0, nrows, 0, src.shape[1], shp, r0, 0)

    def strips(src, dst, sem, s, c0, ncols):
        return pieces(src, dst, sem, _al(s * _GD, _GD), _GD, w0 + c0, ncols, cfg["kv"], 0, c0)

    def start(lo, hi):
        for (src, r0, c0, dst, dr0, dc0, r, c, rows, cols, sem), prio in _merge(
                [(p, _LO) for p in lo], [(p, _HI) for p in hi]):
            pltpu.make_async_copy(
                src.at[pl.ds(r0 + r, rows), pl.ds(c0 + c, cols)],
                dst.at[pl.ds(dr0 + r, rows), pl.ds(dc0 + c, cols)],
                sems.at[sem]).start(priority=prio)

    def wait_all(ref, sem):
        pltpu.make_async_copy(ref, ref, sems.at[sem]).wait()

    def start_k_half(s, h):
        wo = pieces(wo_hbm, wo_b.at[s], s_wo + s % 2, _al(s * _GD + h * _DH, _DH), _DH,
                    0, d_model, cfg["wo"], h * _DH, 0)
        wg = rows_of(wg_hbm, wg_b, s_g, _al(s * rg, rg), rg, cfg["wgu"])
        wu = rows_of(wu_hbm, wu_b, s_u, _al(s * uk, uk), uk, cfg["wgu"])
        start(_half(strips(kt_hbm, k_b.at[s % 2], s_k + s % 2, s, 0, win), h),
              _merge(wo, _half(wg, h) + _half(wu, h)))

    def start_vlast_half(h):
        lo = []
        for j in range(nvb):
            lo += strips(vt_hbm, v_b.at[last], s_v + j, last, j * cw, cw)
        start(_half(lo, h), rows_of(wu_hbm, wu_b, s_u, ub + h * u0, (u0, u1)[h], cfg["wgu"]))

    def start_tail():
        lo = []
        for j in range(len(dsplit)):
            lo += rows_of(wd_hbm, wd_b, s_d + j, sum(dsplit[:j]), dsplit[j], cfg["wd"])
        r = ub + u0 + u1
        start(lo, rows_of(wu_hbm, wu_b, s_u, r, d_model - r, cfg["wgu"]))

    cx = pltpu.make_async_copy(x_hbm, x_b, sems.at[s_x])
    cc = pltpu.make_async_copy(c_hbm, c_b, sems.at[s_c])
    cx.start(priority=_HI)
    cc.start(priority=_HI)

    def phase_a(u, carry):
        start(strips(vt_hbm, v_b.at[u], s_v0, u, 0, win),
              rows_of(wm_hbm, wm_b, s_wm, _al(u * ra, ra), ra, cfg["wm"]))
        return carry
    lax.fori_loop(0, na, phase_a, 0)

    def phase_b(u, carry):
        start(strips(vt_hbm, v_b.at[u], s_v0, u, 0, win),
              rows_of(wq_hbm, wq_b, s_wq, _al((u - na) * rb, rb), rb, cfg["wq"]))

        @pl.when(u == na)
        def _():
            cc.wait()
            cv = jnp.broadcast_to(c_b[...].astype(f32), (_M, d_model))
            sc = (cv * jax.nn.sigmoid(cv)).astype(bf16)
            wait_all(wm_b, s_wm)
            mod_s[...] = jnp.dot(sc, wm_b[...], preferred_element_type=f32)
        return carry
    lax.fori_loop(na, last, phase_b, 0)

    def mod(i):
        return mod_s[:, pl.ds(i * d_model, d_model)]

    start_k_half(0, 0)
    cx.wait()
    x = jnp.broadcast_to(x_b[...].astype(f32), (_M, d_model))
    h = (_layernorm(x) * (1.0 + mod(1)) + mod(0)).astype(bf16)
    wait_all(wq_b, s_wq)
    q = jnp.dot(h, wq_b[...], preferred_element_type=f32)
    diag = _diag()
    for s in range(_NS):
        q_s[s] = jnp.where(diag, q[:, s * _GD:(s + 1) * _GD], 0.0).astype(bf16)
    acc_s[...] = jnp.zeros_like(acc_s)
    start_k_half(0, 1)
    start_k_half(1, 0)
    wait_all(v_b.at[pl.ds(0, last)], s_v0)

    def stage(s, carry):
        slot = s % 2

        @pl.when(s < last)
        def _():
            start_k_half(s + 1, 1)

        @pl.when(s == last)
        def _():
            start_vlast_half(1)

        wait_all(k_b.at[slot], s_k + slot)
        wait_all(wo_b.at[s], s_wo + slot)
        sco = jnp.dot(q_s[s], k_b[slot], preferred_element_type=f32) * (_DH ** -0.5)
        e = jnp.exp(sco - jnp.max(sco, axis=-1, keepdims=True))
        l_s[...] = jnp.broadcast_to(jnp.sum(e, axis=-1, keepdims=True), l_s.shape)
        e_s[...] = e.astype(bf16)

        @pl.when(s < last - 1)
        def _():
            start_k_half(s + 2, 0)

        @pl.when(s == last - 1)
        def _():
            start_vlast_half(0)

        @pl.when(s == last)
        def _():
            start_tail()

        for j in range(nvb):
            @pl.when(s == last)
            def _():
                wait_all(v_b.at[last, :, pl.ds(j * cw, cw)], s_v + j)
            o = lax.dot_general(e_s[:, pl.ds(j * cw, cw)], v_b[s, :, pl.ds(j * cw, cw)],
                                (((1,), (1,)), ((), ())), preferred_element_type=f32)
            if j > 0:
                o = o + o_s[...]
            if j < nvb - 1:
                o_s[...] = o
        o = jnp.where(_diag(), o / l_s[:, 0:1], 0.0).astype(bf16)
        acc_s[...] += jnp.dot(o, wo_b[s], preferred_element_type=f32)
        return carry
    lax.fori_loop(0, _NS, stage, 0)

    wait_all(wg_b, s_g)
    wait_all(wu_b, s_u)
    attn = jnp.sum(acc_s[...], axis=0, keepdims=True)
    x = jnp.broadcast_to(x_b[...].astype(f32), (_M, d_model))
    x1 = x + mod(2) * attn
    h2 = (_layernorm(x1) * (1.0 + mod(4)) + mod(3)).astype(bf16)
    gg = jnp.dot(h2, wg_b[...], preferred_element_type=f32)
    uu = jnp.dot(h2, wu_b[...], preferred_element_type=f32)
    hh = (gg * uu).astype(bf16)
    r = 0
    for j, n in enumerate(dsplit[:-1]):
        wait_all(wd_b.at[pl.ds(r, n), :], s_d + j)
        y = jnp.dot(hh[:, r:r + n], wd_b[pl.ds(r, n), :], preferred_element_type=f32)
        acc_s[...] = y if j == 0 else y + acc_s[...]
        if j == 0:
            ht = hh[:, d_ff - vr:].astype(f32).T
            hb_s[...] = jnp.broadcast_to(ht[:, 0:1], hb_s.shape)
        r += n
    wait_all(wd_b.at[pl.ds(r, vr), :], s_d + len(dsplit) - 1)
    w = wd_b[pl.ds(r, vr), :].astype(f32)
    hb = hb_s[...]
    part = jnp.concatenate(
        [jnp.sum((w[:, c:c + 128] * hb).reshape(vr // 8, 8, 128), axis=0)
         for c in range(0, d_model, 128)], axis=1)
    y = jnp.sum(part, axis=0, keepdims=True) + acc_s[0:1, :]
    o_ref[...] = (x1[0:1] + mod(5)[0:1] * y).astype(o_ref.dtype)


def _build(cfg, A_x, A_k_cache, A_v_cache, A_wq, A_wo, B_w_gate, B_w_up, B_w_down, c, w_mod,
           interpret=False):
    b, sq, d_model = A_x.shape
    _, hkv, sk, dh = A_k_cache.shape
    assert b == 1 and sq == 1 and hkv == _H and dh == _DH
    d_ff = B_w_gate.shape[1]
    win = min(4096, max(256, sk // 4))
    f32, bf16 = jnp.float32, jnp.bfloat16

    kt = jnp.transpose(A_k_cache, (0, 1, 3, 2)).reshape(_H * _DH, sk)
    vt = jnp.transpose(A_v_cache, (0, 1, 3, 2)).reshape(_H * _DH, sk)

    out = pl.pallas_call(
        functools.partial(_kernel, cfg=cfg, d_model=d_model, d_ff=d_ff, sk=sk, win=win),
        out_shape=jax.ShapeDtypeStruct((1, d_model), A_x.dtype),
        in_specs=[pl.BlockSpec(memory_space=pl.ANY)] * 10,
        out_specs=pl.BlockSpec(memory_space=pltpu.VMEM),
        scratch_shapes=[
            pltpu.VMEM((1, d_model), bf16),
            pltpu.VMEM((1, d_model), bf16),
            pltpu.VMEM((d_model, 6 * d_model), bf16),
            pltpu.VMEM((2, _GD, win), bf16),
            pltpu.VMEM((_NS, _GD, win), bf16),
            pltpu.VMEM((d_model, _H * _DH), bf16),
            pltpu.VMEM((_NS, _GD, d_model), bf16),
            pltpu.VMEM((d_model, d_ff), bf16),
            pltpu.VMEM((d_model, d_ff), bf16),
            pltpu.VMEM((d_ff, d_model), bf16),
            pltpu.VMEM((_M, 6 * d_model), f32),
            pltpu.VMEM((_NS, _M, _GD), bf16),
            pltpu.VMEM((_M, d_model), f32),
            pltpu.VMEM((_M, win), bf16),
            pltpu.VMEM((_M, 128), f32),
            pltpu.VMEM((_M, _GD), f32),
            pltpu.VMEM((cfg["dsplit"][-1], 128), f32),
            pltpu.SemaphoreType.DMA((11 + cfg["nvb"] + len(cfg["dsplit"]),)),
        ],
        compiler_params=pltpu.CompilerParams(
            vmem_limit_bytes=110 * 1024 * 1024,
            disable_bounds_checks=True,
            disable_semaphore_checks=True),
        interpret=interpret,
    )(A_x.reshape(1, d_model), c, kt, vt, A_wq, A_wo, B_w_gate, B_w_up, B_w_down, w_mod)
    return out.reshape(1, 1, d_model)


@jax.jit
def pallas_adaLN_cond__sliding_block_cached__glu_gated_bilinear__decode_kernel(
    A_x: jax.Array,
    A_k_cache: jax.Array,
    A_v_cache: jax.Array,
    A_wq: jax.Array,
    A_wo: jax.Array,
    B_x: jax.Array,
    B_w_gate: jax.Array,
    B_w_up: jax.Array,
    B_w_down: jax.Array,
    c: jax.Array,
    w_mod: jax.Array,
):
    del B_x
    return _build(_CFG, A_x, A_k_cache, A_v_cache, A_wq, A_wo, B_w_gate, B_w_up, B_w_down,
                  c, w_mod)
```

```python
import functools

import jax
import jax.numpy as jnp
from jax import lax
import jax.experimental.pallas as pl
import jax.experimental.pallas.tpu as pltpu

_H = 32
_DH = 192
_GD = 2 * _DH
_NS = _H // 2
_EPS = 1e-5
_M = 8
_HI, _LO = 0, 1

_CFG = dict(
    nvb=4,
    dmxu=(896, 384, 128),
    dvpu=(80, 32, 16),
    kv=(192, 128),
    wm=(8, 768), wq=(8, 768), wo=(8, 640), wgu=(8, 768), wd=(64, 640),
    na=5,
    wu_k=24,
    wu_v=(88, 88),
)


def _layernorm(x):
    m = jnp.mean(x, axis=-1, keepdims=True)
    d = x - m
    v = jnp.mean(d * d, axis=-1, keepdims=True)
    return d / jnp.sqrt(v + _EPS)


def _merge(*lists):
    items = []
    for li, lst in enumerate(lists):
        for i, x in enumerate(lst):
            items.append(((i + 0.5) / len(lst), li, i, x))
    items.sort(key=lambda t: t[:3])
    return [t[3] for t in items]


def _half(lst, h):
    n = len(lst) // 2
    return lst[:n] if h == 0 else lst[n:]


def _al(v, k):
    return v if isinstance(v, int) else pl.multiple_of(v, k)


def _diag():
    row = lax.broadcasted_iota(jnp.int32, (_M, _GD), 0)
    col = lax.broadcasted_iota(jnp.int32, (_M, _GD), 1)
    return (col >= row * _DH) & (col < (row + 1) * _DH)


def _kernel(x_hbm, c_hbm, kt_hbm, vt_hbm, wq_hbm, wo_hbm, wg_hbm, wu_hbm, wd_hbm, wm_hbm,
            o_ref,
            x_b, c_b, wm_b, k_b, v_b, wq_b, wo_b, wg_b, wu_b, wd_b,
            mod_s, q_s, acc_s, e_s, l_s, o_s, hb_s,
            sems,
            *, cfg, d_model, d_ff, sk, win):
    f32, bf16 = jnp.float32, jnp.bfloat16
    nvb, dmxu, dvpu, na = cfg["nvb"], cfg["dmxu"], cfg["dvpu"], cfg["na"]
    dsplit = dmxu + dvpu
    last = _NS - 1
    cw = win // nvb
    w0 = sk - win
    ra, rb, rg = d_model // na, d_model // (last - na), d_model // _NS
    uk = cfg["wu_k"]
    u0, u1 = cfg["wu_v"]
    ub = uk * _NS
    vr = sum(dvpu)
    assert sum(dsplit) == d_ff and vr == 128

    s_x, s_c, s_wm, s_wq, s_g, s_u, s_v0, s_k, s_wo, s_v = 0, 1, 2, 3, 4, 5, 6, 7, 9, 11
    s_d = s_v + nvb

    def pieces(src, dst, sem, r0, nrows, c0, ncols, shp, dr0, dc0):
        rows, cols = shp
        assert nrows % rows == 0 and ncols % cols == 0, (nrows, ncols, shp)
        return [(src, r0, c0, dst, dr0, dc0, r, c, rows, cols, sem)
                for r in range(0, nrows, rows) for c in range(0, ncols, cols)]

    def rows_of(src, dst, sem, r0, nrows, shp):
        return pieces(src, dst, sem, r0, nrows, 0, src.shape[1], shp, r0, 0)

    def strips(src, dst, sem, s, c0, ncols):
        return pieces(src, dst, sem, _al(s * _GD, _GD), _GD, w0 + c0, ncols, cfg["kv"], 0, c0)

    def start(lo, hi):
        for (src, r0, c0, dst, dr0, dc0, r, c, rows, cols, sem), prio in _merge(
                [(p, _LO) for p in lo], [(p, _HI) for p in hi]):
            pltpu.make_async_copy(
                src.at[pl.ds(r0 + r, rows), pl.ds(c0 + c, cols)],
                dst.at[pl.ds(dr0 + r, rows), pl.ds(dc0 + c, cols)],
                sems.at[sem]).start(priority=prio)

    def wait_all(ref, sem):
        pltpu.make_async_copy(ref, ref, sems.at[sem]).wait()

    def start_k_half(s, h):
        wo = pieces(wo_hbm, wo_b.at[s], s_wo + s % 2, _al(s * _GD + h * _DH, _DH), _DH,
                    0, d_model, cfg["wo"], h * _DH, 0)
        wg = rows_of(wg_hbm, wg_b, s_g, _al(s * rg, rg), rg, cfg["wgu"])
        wu = rows_of(wu_hbm, wu_b, s_u, _al(s * uk, uk), uk, cfg["wgu"])
        start(_half(strips(kt_hbm, k_b.at[s % 2], s_k + s % 2, s, 0, win), h),
              _merge(wo, _half(wg, h) + _half(wu, h)))

    def start_vlast_half(h):
        lo = []
        for j in range(nvb):
            lo += strips(vt_hbm, v_b.at[last], s_v + j, last, j * cw, cw)
        start(_half(lo, h), rows_of(wu_hbm, wu_b, s_u, ub + h * u0, (u0, u1)[h], cfg["wgu"]))

    def start_tail():
        lo = []
        for j in range(len(dsplit)):
            n = dsplit[j]
            shp = cfg["wd"] if j < len(dmxu) else (n, d_model)
            lo += rows_of(wd_hbm, wd_b, s_d + j, sum(dsplit[:j]), n, shp)
        r = ub + u0 + u1
        start(lo, rows_of(wu_hbm, wu_b, s_u, r, d_model - r, cfg["wgu"]))

    cx = pltpu.make_async_copy(x_hbm, x_b, sems.at[s_x])
    cc = pltpu.make_async_copy(c_hbm, c_b, sems.at[s_c])
    cx.start(priority=_HI)
    cc.start(priority=_HI)

    def phase_a(u, carry):
        start(strips(vt_hbm, v_b.at[u], s_v0, u, 0, win),
              rows_of(wm_hbm, wm_b, s_wm, _al(u * ra, ra), ra, cfg["wm"]))
        return carry
    lax.fori_loop(0, na, phase_a, 0)

    def phase_b(u, carry):
        start(strips(vt_hbm, v_b.at[u], s_v0, u, 0, win),
              rows_of(wq_hbm, wq_b, s_wq, _al((u - na) * rb, rb), rb, cfg["wq"]))

        @pl.when(u == na)
        def _():
            cc.wait()
            cv = jnp.broadcast_to(c_b[...].astype(f32), (_M, d_model))
            sc = (cv * jax.nn.sigmoid(cv)).astype(bf16)
            wait_all(wm_b, s_wm)
            mod_s[...] = jnp.dot(sc, wm_b[...], preferred_element_type=f32)
        return carry
    lax.fori_loop(na, last, phase_b, 0)

    def mod(i):
        return mod_s[:, pl.ds(i * d_model, d_model)]

    start_k_half(0, 0)
    cx.wait()
    x = jnp.broadcast_to(x_b[...].astype(f32), (_M, d_model))
    h = (_layernorm(x) * (1.0 + mod(1)) + mod(0)).astype(bf16)
    wait_all(wq_b, s_wq)
    q = jnp.dot(h, wq_b[...], preferred_element_type=f32)
    diag = _diag()
    for s in range(_NS):
        q_s[s] = jnp.where(diag, q[:, s * _GD:(s + 1) * _GD], 0.0).astype(bf16)
    acc_s[...] = jnp.zeros_like(acc_s)
    start_k_half(0, 1)
    start_k_half(1, 0)
    wait_all(v_b.at[pl.ds(0, last)], s_v0)

    def stage(s, carry):
        slot = s % 2

        @pl.when(s < last)
        def _():
            start_k_half(s + 1, 1)

        @pl.when(s == last)
        def _():
            start_vlast_half(1)

        wait_all(k_b.at[slot], s_k + slot)
        wait_all(wo_b.at[s], s_wo + slot)
        sco = jnp.dot(q_s[s], k_b[slot], preferred_element_type=f32) * (_DH ** -0.5)
        e = jnp.exp(sco - jnp.max(sco, axis=-1, keepdims=True))
        l_s[...] = jnp.broadcast_to(jnp.sum(e, axis=-1, keepdims=True), l_s.shape)
        e_s[...] = e.astype(bf16)

        @pl.when(s < last - 1)
        def _():
            start_k_half(s + 2, 0)

        @pl.when(s == last - 1)
        def _():
            start_vlast_half(0)

        @pl.when(s == last)
        def _():
            start_tail()

        for j in range(nvb):
            @pl.when(s == last)
            def _():
                wait_all(v_b.at[last, :, pl.ds(j * cw, cw)], s_v + j)
            o = lax.dot_general(e_s[:, pl.ds(j * cw, cw)], v_b[s, :, pl.ds(j * cw, cw)],
                                (((1,), (1,)), ((), ())), preferred_element_type=f32)
            if j > 0:
                o = o + o_s[...]
            if j < nvb - 1:
                o_s[...] = o
        o = jnp.where(_diag(), o / l_s[:, 0:1], 0.0).astype(bf16)
        acc_s[...] += jnp.dot(o, wo_b[s], preferred_element_type=f32)
        return carry
    lax.fori_loop(0, _NS, stage, 0)

    wait_all(wg_b, s_g)
    wait_all(wu_b, s_u)
    attn = jnp.sum(acc_s[...], axis=0, keepdims=True)
    x = jnp.broadcast_to(x_b[...].astype(f32), (_M, d_model))
    x1 = x + mod(2) * attn
    h2 = (_layernorm(x1) * (1.0 + mod(4)) + mod(3)).astype(bf16)
    gg = jnp.dot(h2, wg_b[...], preferred_element_type=f32)
    uu = jnp.dot(h2, wu_b[...], preferred_element_type=f32)
    hh = (gg * uu).astype(bf16)
    r = 0
    for j, n in enumerate(dmxu):
        wait_all(wd_b.at[pl.ds(r, n), :], s_d + j)
        y = jnp.dot(hh[:, r:r + n], wd_b[pl.ds(r, n), :], preferred_element_type=f32)
        acc_s[...] = y if j == 0 else y + acc_s[...]
        if j == 0:
            ht = hh[:, d_ff - vr:].astype(f32).T
            hb_s[...] = jnp.broadcast_to(ht[:, 0:1], hb_s.shape)
        r += n
    part = None
    for j, n in enumerate(dvpu):
        wait_all(wd_b.at[pl.ds(r, n), :], s_d + len(dmxu) + j)
        w = wd_b[pl.ds(r, n), :].astype(f32)
        hb = hb_s[pl.ds(r - (d_ff - vr), n), :]
        pj = jnp.concatenate(
            [jnp.sum((w[:, c:c + 128] * hb).reshape(n // 8, 8, 128), axis=0)
             for c in range(0, d_model, 128)], axis=1)
        part = pj if part is None else part + pj
        r += n
    y = jnp.sum(part, axis=0, keepdims=True) + acc_s[0:1, :]
    o_ref[...] = (x1[0:1] + mod(5)[0:1] * y).astype(o_ref.dtype)


def _build(cfg, A_x, A_k_cache, A_v_cache, A_wq, A_wo, B_w_gate, B_w_up, B_w_down, c, w_mod,
           interpret=False):
    b, sq, d_model = A_x.shape
    _, hkv, sk, dh = A_k_cache.shape
    assert b == 1 and sq == 1 and hkv == _H and dh == _DH
    d_ff = B_w_gate.shape[1]
    win = min(4096, max(256, sk // 4))
    f32, bf16 = jnp.float32, jnp.bfloat16

    kt = jnp.transpose(A_k_cache, (0, 1, 3, 2)).reshape(_H * _DH, sk)
    vt = jnp.transpose(A_v_cache, (0, 1, 3, 2)).reshape(_H * _DH, sk)

    out = pl.pallas_call(
        functools.partial(_kernel, cfg=cfg, d_model=d_model, d_ff=d_ff, sk=sk, win=win),
        out_shape=jax.ShapeDtypeStruct((1, d_model), A_x.dtype),
        in_specs=[pl.BlockSpec(memory_space=pl.ANY)] * 10,
        out_specs=pl.BlockSpec(memory_space=pltpu.VMEM),
        scratch_shapes=[
            pltpu.VMEM((1, d_model), bf16),
            pltpu.VMEM((1, d_model), bf16),
            pltpu.VMEM((d_model, 6 * d_model), bf16),
            pltpu.VMEM((2, _GD, win), bf16),
            pltpu.VMEM((_NS, _GD, win), bf16),
            pltpu.VMEM((d_model, _H * _DH), bf16),
            pltpu.VMEM((_NS, _GD, d_model), bf16),
            pltpu.VMEM((d_model, d_ff), bf16),
            pltpu.VMEM((d_model, d_ff), bf16),
            pltpu.VMEM((d_ff, d_model), bf16),
            pltpu.VMEM((_M, 6 * d_model), f32),
            pltpu.VMEM((_NS, _M, _GD), bf16),
            pltpu.VMEM((_M, d_model), f32),
            pltpu.VMEM((_M, win), bf16),
            pltpu.VMEM((_M, 128), f32),
            pltpu.VMEM((_M, _GD), f32),
            pltpu.VMEM((sum(cfg["dvpu"]), 128), f32),
            pltpu.SemaphoreType.DMA((11 + cfg["nvb"] + len(cfg["dmxu"] + cfg["dvpu"]),)),
        ],
        compiler_params=pltpu.CompilerParams(
            vmem_limit_bytes=110 * 1024 * 1024,
            disable_bounds_checks=True,
            disable_semaphore_checks=True),
        interpret=interpret,
    )(A_x.reshape(1, d_model), c, kt, vt, A_wq, A_wo, B_w_gate, B_w_up, B_w_down, w_mod)
    return out.reshape(1, 1, d_model)


@jax.jit
def pallas_adaLN_cond__sliding_block_cached__glu_gated_bilinear__decode_kernel(
    A_x: jax.Array,
    A_k_cache: jax.Array,
    A_v_cache: jax.Array,
    A_wq: jax.Array,
    A_wo: jax.Array,
    B_x: jax.Array,
    B_w_gate: jax.Array,
    B_w_up: jax.Array,
    B_w_down: jax.Array,
    c: jax.Array,
    w_mod: jax.Array,
):
    del B_x
    return _build(_CFG, A_x, A_k_cache, A_v_cache, A_wq, A_wo, B_w_gate, B_w_up, B_w_down,
                  c, w_mod)
```

```python
import functools

import jax
import jax.numpy as jnp
from jax import lax
import jax.experimental.pallas as pl
import jax.experimental.pallas.tpu as pltpu

_H = 32
_DH = 192
_GD = 2 * _DH
_NS = _H // 2
_EPS = 1e-5
_M = 8
_HI, _LO = 0, 1

_CFG = dict(
    nvb=4,
    wdr=((384, 24, "A"), (384, 24, "A"), (384, 24, "B"), (192, 24, "B"),
         (144, 8, "C"), (32, 8, "C"), (16, 8, "C")),
    mxu_order=((0, 2), (3, 1)),
    kv=(192, 128),
    wm=(8, 768), wq=(8, 768), wo=(8, 640), wgu=(8, 768),
    na=5,
    wu_k=24,
    wu_v=(88, 88),
)


def _layernorm(x):
    m = jnp.mean(x, axis=-1, keepdims=True)
    d = x - m
    v = jnp.mean(d * d, axis=-1, keepdims=True)
    return d / jnp.sqrt(v + _EPS)


def _merge(*lists):
    items = []
    for li, lst in enumerate(lists):
        for i, x in enumerate(lst):
            items.append(((i + 0.5) / len(lst), li, i, x))
    items.sort(key=lambda t: t[:3])
    return [t[3] for t in items]


def _half(lst, h):
    n = len(lst) // 2
    return lst[:n] if h == 0 else lst[n:]


def _al(v, k):
    return v if isinstance(v, int) else pl.multiple_of(v, k)


def _diag():
    row = lax.broadcasted_iota(jnp.int32, (_M, _GD), 0)
    col = lax.broadcasted_iota(jnp.int32, (_M, _GD), 1)
    return (col >= row * _DH) & (col < (row + 1) * _DH)


def _kernel(x_hbm, c_hbm, kt_hbm, vt_hbm, wq_hbm, wo_hbm, wg_hbm, wu_hbm, wd_hbm, wm_hbm,
            o_ref,
            x_b, c_b, wm_b, k_b, v_b, wq_b, wo_b, wg_b, wu_b, wd_b,
            mod_s, q_s, acc_s, e_s, l_s, o_s, hb_s,
            sems,
            *, cfg, d_model, d_ff, sk, win):
    f32, bf16 = jnp.float32, jnp.bfloat16
    nvb, wdr, na = cfg["nvb"], cfg["wdr"], cfg["na"]
    wd0 = [sum(t[0] for t in wdr[:j]) for j in range(len(wdr))]
    vpu = [j for j in range(len(wdr)) if not any(j in g for g in cfg["mxu_order"])]
    last = _NS - 1
    cw = win // nvb
    w0 = sk - win
    ra, rb, rg = d_model // na, d_model // (last - na), d_model // _NS
    uk = cfg["wu_k"]
    u0, u1 = cfg["wu_v"]
    ub = uk * _NS
    vr = sum(wdr[j][0] for j in vpu)
    vrp = hb_s.shape[0]
    assert sum(t[0] for t in wdr) == d_ff and wd0[vpu[0]] == d_ff - vr and vr <= vrp

    s_x, s_c, s_wm, s_wq, s_g, s_u, s_v0, s_k, s_wo, s_v = 0, 1, 2, 3, 4, 5, 6, 7, 9, 11
    s_d = s_v + nvb

    def pieces(src, dst, sem, r0, nrows, c0, ncols, shp, dr0, dc0):
        rows, cols = shp
        assert nrows % rows == 0 and ncols % cols == 0, (nrows, ncols, shp)
        return [(src, r0, c0, dst, dr0, dc0, r, c, rows, cols, sem)
                for r in range(0, nrows, rows) for c in range(0, ncols, cols)]

    def rows_of(src, dst, sem, r0, nrows, shp):
        return pieces(src, dst, sem, r0, nrows, 0, src.shape[1], shp, r0, 0)

    def strips(src, dst, sem, s, c0, ncols):
        return pieces(src, dst, sem, _al(s * _GD, _GD), _GD, w0 + c0, ncols, cfg["kv"], 0, c0)

    def start(lo, hi):
        for (src, r0, c0, dst, dr0, dc0, r, c, rows, cols, sem), prio in _merge(
                [(p, _LO) for p in lo], [(p, _HI) for p in hi]):
            pltpu.make_async_copy(
                src.at[pl.ds(r0 + r, rows), pl.ds(c0 + c, cols)],
                dst.at[pl.ds(dr0 + r, rows), pl.ds(dc0 + c, cols)],
                sems.at[sem]).start(priority=prio)

    def wait_all(ref, sem):
        pltpu.make_async_copy(ref, ref, sems.at[sem]).wait()

    def start_k_half(s, h):
        wo = pieces(wo_hbm, wo_b.at[s], s_wo + s % 2, _al(s * _GD + h * _DH, _DH), _DH,
                    0, d_model, cfg["wo"], h * _DH, 0)
        wg = rows_of(wg_hbm, wg_b, s_g, _al(s * rg, rg), rg, cfg["wgu"])
        wu = rows_of(wu_hbm, wu_b, s_u, _al(s * uk, uk), uk, cfg["wgu"])
        start(_half(strips(kt_hbm, k_b.at[s % 2], s_k + s % 2, s, 0, win), h),
              _merge(wo, _half(wg, h) + _half(wu, h)))

    def start_vlast_half(h):
        lo = []
        for j in range(nvb):
            lo += strips(vt_hbm, v_b.at[last], s_v + j, last, j * cw, cw)
        start(_half(lo, h), rows_of(wu_hbm, wu_b, s_u, ub + h * u0, (u0, u1)[h], cfg["wgu"]))

    def wd_stream(name):
        out = []
        for j, (n, p, st) in enumerate(wdr):
            if st == name:
                out += rows_of(wd_hbm, wd_b, s_d + j, wd0[j], n, (p, d_model))
        return out

    def start_tail():
        r = ub + u0 + u1
        start(wd_stream("A"), rows_of(wu_hbm, wu_b, s_u, r, d_model - r, cfg["wgu"]))

    cx = pltpu.make_async_copy(x_hbm, x_b, sems.at[s_x])
    cc = pltpu.make_async_copy(c_hbm, c_b, sems.at[s_c])
    cx.start(priority=_HI)
    cc.start(priority=_HI)

    def phase_a(u, carry):
        start(strips(vt_hbm, v_b.at[u], s_v0, u, 0, win),
              rows_of(wm_hbm, wm_b, s_wm, _al(u * ra, ra), ra, cfg["wm"]))
        return carry
    lax.fori_loop(0, na, phase_a, 0)

    def phase_b(u, carry):
        start(strips(vt_hbm, v_b.at[u], s_v0, u, 0, win),
              rows_of(wq_hbm, wq_b, s_wq, _al((u - na) * rb, rb), rb, cfg["wq"]))

        @pl.when(u == na)
        def _():
            cc.wait()
            cv = jnp.broadcast_to(c_b[...].astype(f32), (_M, d_model))
            sc = (cv * jax.nn.sigmoid(cv)).astype(bf16)
            wait_all(wm_b, s_wm)
            mod_s[...] = jnp.dot(sc, wm_b[...], preferred_element_type=f32)
        return carry
    lax.fori_loop(na, last, phase_b, 0)

    def mod(i):
        return mod_s[:, pl.ds(i * d_model, d_model)]

    start_k_half(0, 0)
    cx.wait()
    x = jnp.broadcast_to(x_b[...].astype(f32), (_M, d_model))
    h = (_layernorm(x) * (1.0 + mod(1)) + mod(0)).astype(bf16)
    wait_all(wq_b, s_wq)
    q = jnp.dot(h, wq_b[...], preferred_element_type=f32)
    diag = _diag()
    for s in range(_NS):
        q_s[s] = jnp.where(diag, q[:, s * _GD:(s + 1) * _GD], 0.0).astype(bf16)
    acc_s[...] = jnp.zeros_like(acc_s)
    start_k_half(0, 1)
    start_k_half(1, 0)
    wait_all(v_b.at[pl.ds(0, last)], s_v0)

    def stage(s, carry):
        slot = s % 2

        @pl.when(s < last)
        def _():
            start_k_half(s + 1, 1)

        @pl.when(s == last)
        def _():
            start_vlast_half(1)

        wait_all(k_b.at[slot], s_k + slot)
        wait_all(wo_b.at[s], s_wo + slot)
        sco = jnp.dot(q_s[s], k_b[slot], preferred_element_type=f32) * (_DH ** -0.5)
        e = jnp.exp(sco - jnp.max(sco, axis=-1, keepdims=True))
        l_s[...] = jnp.broadcast_to(jnp.sum(e, axis=-1, keepdims=True), l_s.shape)
        e_s[...] = e.astype(bf16)

        @pl.when(s < last - 1)
        def _():
            start_k_half(s + 2, 0)

        @pl.when(s == last - 1)
        def _():
            start_vlast_half(0)

        @pl.when(s == last)
        def _():
            start_tail()

        for j in range(nvb):
            @pl.when(s == last)
            def _():
                wait_all(v_b.at[last, :, pl.ds(j * cw, cw)], s_v + j)
                if j == nvb - 1:
                    start(wd_stream("C"), wd_stream("B"))
            o = lax.dot_general(e_s[:, pl.ds(j * cw, cw)], v_b[s, :, pl.ds(j * cw, cw)],
                                (((1,), (1,)), ((), ())), preferred_element_type=f32)
            if j > 0:
                o = o + o_s[...]
            if j < nvb - 1:
                o_s[...] = o
        o = jnp.where(_diag(), o / l_s[:, 0:1], 0.0).astype(bf16)
        acc_s[...] += jnp.dot(o, wo_b[s], preferred_element_type=f32)
        return carry
    lax.fori_loop(0, _NS, stage, 0)

    wait_all(wg_b, s_g)
    wait_all(wu_b, s_u)
    attn = jnp.sum(acc_s[...], axis=0, keepdims=True)
    x = jnp.broadcast_to(x_b[...].astype(f32), (_M, d_model))
    x1 = x + mod(2) * attn
    h2 = (_layernorm(x1) * (1.0 + mod(4)) + mod(3)).astype(bf16)
    gg = jnp.dot(h2, wg_b[...], preferred_element_type=f32)
    uu = jnp.dot(h2, wu_b[...], preferred_element_type=f32)
    hh = (gg * uu).astype(bf16)
    for gi, grp in enumerate(cfg["mxu_order"]):
        for j in grp:
            wait_all(wd_b.at[pl.ds(wd0[j], wdr[j][0]), :], s_d + j)
        y = None if gi == 0 else acc_s[...]
        for j in grp:
            r, n = wd0[j], wdr[j][0]
            t = jnp.dot(hh[:, r:r + n], wd_b[pl.ds(r, n), :], preferred_element_type=f32)
            y = t if y is None else y + t
        acc_s[...] = y
        if gi == 0:
            ht = hh[:, d_ff - vrp:].astype(f32).T
            hb_s[...] = jnp.broadcast_to(ht[:, 0:1], hb_s.shape)
    part = None
    for j in vpu:
        r, n = wd0[j], wdr[j][0]
        wait_all(wd_b.at[pl.ds(r, n), :], s_d + j)
        w = wd_b[pl.ds(r, n), :].astype(f32)
        hb = hb_s[pl.ds(r - (d_ff - vrp), n), :]
        pj = jnp.concatenate(
            [jnp.sum((w[:, c:c + 128] * hb).reshape(n // 8, 8, 128), axis=0)
             for c in range(0, d_model, 128)], axis=1)
        part = pj if part is None else part + pj
    y = jnp.sum(part, axis=0, keepdims=True) + acc_s[0:1, :]
    o_ref[...] = (x1[0:1] + mod(5)[0:1] * y).astype(o_ref.dtype)


def _build(cfg, A_x, A_k_cache, A_v_cache, A_wq, A_wo, B_w_gate, B_w_up, B_w_down, c, w_mod,
           interpret=False):
    b, sq, d_model = A_x.shape
    _, hkv, sk, dh = A_k_cache.shape
    assert b == 1 and sq == 1 and hkv == _H and dh == _DH
    d_ff = B_w_gate.shape[1]
    win = min(4096, max(256, sk // 4))
    f32, bf16 = jnp.float32, jnp.bfloat16

    kt = jnp.transpose(A_k_cache, (0, 1, 3, 2)).reshape(_H * _DH, sk)
    vt = jnp.transpose(A_v_cache, (0, 1, 3, 2)).reshape(_H * _DH, sk)

    out = pl.pallas_call(
        functools.partial(_kernel, cfg=cfg, d_model=d_model, d_ff=d_ff, sk=sk, win=win),
        out_shape=jax.ShapeDtypeStruct((1, d_model), A_x.dtype),
        in_specs=[pl.BlockSpec(memory_space=pl.ANY)] * 10,
        out_specs=pl.BlockSpec(memory_space=pltpu.VMEM),
        scratch_shapes=[
            pltpu.VMEM((1, d_model), bf16),
            pltpu.VMEM((1, d_model), bf16),
            pltpu.VMEM((d_model, 6 * d_model), bf16),
            pltpu.VMEM((2, _GD, win), bf16),
            pltpu.VMEM((_NS, _GD, win), bf16),
            pltpu.VMEM((d_model, _H * _DH), bf16),
            pltpu.VMEM((_NS, _GD, d_model), bf16),
            pltpu.VMEM((d_model, d_ff), bf16),
            pltpu.VMEM((d_model, d_ff), bf16),
            pltpu.VMEM((d_ff, d_model), bf16),
            pltpu.VMEM((_M, 6 * d_model), f32),
            pltpu.VMEM((_NS, _M, _GD), bf16),
            pltpu.VMEM((_M, d_model), f32),
            pltpu.VMEM((_M, win), bf16),
            pltpu.VMEM((_M, 128), f32),
            pltpu.VMEM((_M, _GD), f32),
            pltpu.VMEM((256, 128), f32),
            pltpu.SemaphoreType.DMA((11 + cfg["nvb"] + len(cfg["wdr"]),)),
        ],
        compiler_params=pltpu.CompilerParams(
            vmem_limit_bytes=110 * 1024 * 1024,
            disable_bounds_checks=True,
            disable_semaphore_checks=True),
        interpret=interpret,
    )(A_x.reshape(1, d_model), c, kt, vt, A_wq, A_wo, B_w_gate, B_w_up, B_w_down, w_mod)
    return out.reshape(1, 1, d_model)


@jax.jit
def pallas_adaLN_cond__sliding_block_cached__glu_gated_bilinear__decode_kernel(
    A_x: jax.Array,
    A_k_cache: jax.Array,
    A_v_cache: jax.Array,
    A_wq: jax.Array,
    A_wo: jax.Array,
    B_x: jax.Array,
    B_w_gate: jax.Array,
    B_w_up: jax.Array,
    B_w_down: jax.Array,
    c: jax.Array,
    w_mod: jax.Array,
):
    del B_x
    return _build(_CFG, A_x, A_k_cache, A_v_cache, A_wq, A_wo, B_w_gate, B_w_up, B_w_down,
                  c, w_mod)
```
